```python
import os as _os
_os.environ.setdefault("JAX_PLATFORMS", "cpu")
import jax
import jax.numpy as jnp

def _softmax(x, axis=-1):
    return jax.nn.softmax(x, axis=axis)
def _gelu(x):
    return jax.nn.gelu(x, approximate=True)
def _silu(x):
    return jax.nn.silu(x)
def _sigmoid(x):
    return jax.nn.sigmoid(x)
def _layernorm(x, axis=-1, eps=1e-5):
    m = jnp.mean(x, axis=axis, keepdims=True)
    v = jnp.var(x, axis=axis, keepdims=True)
    return (x - m) / jnp.sqrt(v + eps)
def _scatter_add(tgt, idx, src, axis=0):
    return tgt.at[idx].add(src)
def _segment_sum(src, seg, n):
    return jax.ops.segment_sum(src, seg, n)
class _Rng:
    def __init__(self, key):
        self._k = key
    def _next(self):
        self._k, sub = jax.random.split(self._k)
        return sub
    def normal(self, shape):
        return jax.random.normal(self._next(), shape, dtype=jnp.bfloat16)
    def randint(self, lo, hi, shape):
        return jax.random.randint(self._next(), shape, lo, hi, dtype=jnp.int32)
    def uniform(self, shape, lo=0.0, hi=1.0):
        return jax.random.uniform(self._next(), shape, jnp.bfloat16, lo, hi)
    def permutation(self, n):
        return jax.random.permutation(self._next(), n)


kernel_name = 'gated_mix__linear_attn_block__sliding_local_dilated__prompt'

def setup_inputs():
    _rng = _Rng(jax.random.key(int.from_bytes(__import__("os").urandom(4), "little")))
    _w = (lambda a: (lambda t: t.astype(jnp.bfloat16) if jnp.issubdtype(t.dtype, jnp.floating) else t)(jnp.asarray(a)))
    def _A_setup():
        B, S, D = 1, 2048, 512
        return {
            "x": _w((lambda *s: _rng.normal(s) * 0.05)(B, S, D)),
            "wqkv": _w((lambda *s: _rng.normal(s) * 1.6)(D, 3 * D)),
            "wo": _w((lambda *s: _rng.normal(s) * 0.8)(D, D)),
        }
    _A_in = _A_setup()

    def _B_setup():
        B, S, D = 1, 2048, 512
        return {
            "x": _w((lambda *s: _rng.normal(s) * 0.05)(B, S, D)),
            "wqkv": _w((lambda *s: _rng.normal(s) * 0.8)(D, 3 * D)),
            "wo": _w((lambda *s: _rng.normal(s) * 0.05)(D, D)),
        }
    _B_in = _B_setup()

    return {
        "A_x": _A_in["x"],
        "A_wqkv": _A_in["wqkv"],
        "A_wo": _A_in["wo"],
        "B_x": _B_in["x"],
        "B_wqkv": _B_in["wqkv"],
        "B_wo": _B_in["wo"],
        "gate_w": _w((lambda *s: _rng.normal(s) * 0.05)(512) * 16.0),
    }

def reference(A_x, A_wqkv, A_wo, B_x, B_wqkv, B_wo, gate_w):
    def _A_ref(x, wqkv, wo):
        B, S, D = x.shape
        H = 32; Dh = D // H
        qkv = (lambda x, *d: x.transpose(*d))((x @ wqkv).reshape(B, S, 3, H, Dh), 2, 0, 3, 1, 4)
        q, k, v = qkv[0], qkv[1], qkv[2]
        phi = lambda t: jnp.where(t > 0, t + 1, jnp.exp(t)) + 1e-6
        pq, pk = phi(q), phi(k)
        kv = jnp.einsum("bhsd,bhse->bhde", pk, v)
        z = jnp.einsum("bhsd->bhd", pk)
        num = jnp.einsum("bhqd,bhde->bhqe", pq, kv)
        den = jnp.einsum("bhqd,bhd->bhq", pq, z)[..., None] + 1e-6
        o = num / den
        return (lambda x, *d: x.transpose(*d))(o, 0, 2, 1, 3).reshape(B, S, D) @ wo

    def _B_ref(x, wqkv, wo):
        B, S, D = x.shape
        H = 32; Dh = D // H
        W, dil = 8, 2
        qkv = (lambda x, *d: x.transpose(*d))((x @ wqkv).reshape(B, S, 3, H, Dh), 2, 0, 3, 1, 4)
        q, k, v = qkv[0], qkv[1], qkv[2]
        scale = Dh ** -0.5
        pos = jnp.arange(S)
        off = jnp.arange(W) * dil
        idx = pos[:, None] - off[None, :]
        mask = idx >= 0
        idx_c = jnp.where(mask, idx, 0).reshape(-1)
        kg = k[:, :, idx_c, :].reshape(B, H, S, W, Dh)
        vg = v[:, :, idx_c, :].reshape(B, H, S, W, Dh)
        logits = jnp.einsum("bhsd,bhswd->bhsw", q, kg) * scale
        logits = jnp.where(mask[None, None, :, :], logits, -1e9)
        attn = _softmax(logits, axis=-1)
        o = jnp.einsum("bhsw,bhswd->bhsd", attn, vg)
        return (lambda x, *d: x.transpose(*d))(o, 0, 2, 1, 3).reshape(B, S, D) @ wo

    x = A_x
    g = _sigmoid((x * gate_w).sum(-1, keepdims=True))
    a = _A_ref(x, A_wqkv, A_wo)
    b = _B_ref(x, B_wqkv, B_wo)
    return g * a + (1 - g) * b
```

```python
import jax
import jax.numpy as jnp
from jax import lax
import jax.experimental.pallas as pl
import jax.experimental.pallas.tpu as pltpu

S, D, H, DH, W = 2048, 512, 32, 16, 8
BM1 = 512
BM = 256
CH = 32
PAD = 16
F32, BF16 = jnp.float32, jnp.bfloat16
NT = (((1,), (1,)), ((), ()))


def _phi(t):
    return jnp.where(t > 0, t + 1.0, jnp.exp(t)) + 1e-6


def _kernel(ax_h, awqkv_h, awo_h, bx_h, bwqkv_h, bwo_h, gw_h, out_h,
            ax, bx, awqkv, awo, bwqkv, bwo, gw, outv,
            wkT, tmpT, wpT, bwop, gacc, zblk, mmat, qs, ks, vs, ob,
            sems, osem):
    cps = [
        pltpu.make_async_copy(awqkv_h, awqkv, sems.at[0]),
        pltpu.make_async_copy(ax_h, ax, sems.at[1]),
        pltpu.make_async_copy(awo_h, awo, sems.at[2]),
        pltpu.make_async_copy(bwqkv_h, bwqkv, sems.at[3]),
        pltpu.make_async_copy(bwo_h, bwo, sems.at[4]),
        pltpu.make_async_copy(gw_h, gw, sems.at[5]),
    ]
    for c in cps:
        c.start()
    cps[0].wait()
    wkT[...] = awqkv[:, D:2 * D].astype(F32).T.astype(BF16)
    cps[1].wait()

    def p1(i, zacc):
        r = pl.multiple_of(i * BM1, BM1)
        xb = ax[pl.ds(r, BM1), :]
        kT = lax.dot_general(wkT[...], xb, NT, preferred_element_type=F32)
        pkT = _phi(kT)
        g = jnp.dot(pkT.astype(BF16), xb, preferred_element_type=F32)

        @pl.when(i == 0)
        def _():
            gacc[...] = g

        @pl.when(i > 0)
        def _():
            gacc[...] += g
        zp = pkT[:, 0:128]
        for j in range(1, BM1 // 128):
            zp = zp + pkT[:, j * 128:(j + 1) * 128]
        return zacc + zp

    zacc = lax.fori_loop(0, S // BM1, p1, jnp.zeros((D, 128), F32))
    z = jnp.sum(zacc, axis=1, keepdims=True)
    cps[2].wait()
    ri = lax.broadcasted_iota(jnp.int32, (128, 128), 0) // DH
    ci = lax.broadcasted_iota(jnp.int32, (128, 128), 1) // DH
    bd = ri == ci
    for j in range(4):
        sl = slice(j * 128, (j + 1) * 128)
        zblk[sl, :] = jnp.where(bd, z[sl, :], 0.0).astype(BF16)
        kv = jnp.dot(gacc[sl, :].astype(BF16), awqkv[:, 2 * D + j * 128:2 * D + (j + 1) * 128],
                     preferred_element_type=F32)
        kv = jnp.where(bd, kv, 0.0).astype(BF16)
        mmat[sl, :] = jnp.dot(kv, awo[sl, :], preferred_element_type=F32).astype(BF16)

    cps[3].wait()
    for t in range(3):
        wt = bwqkv[:, t * D:(t + 1) * D].astype(F32).T
        for j in range(4):
            tmpT[j] = wt[:, j * 128:(j + 1) * 128]
        for d in range(DH):
            for j in range(4):
                wpT[t * D + d * H:t * D + (d + 1) * H, j * 128:(j + 1) * 128] = tmpT[j, pl.ds(d, H, stride=DH), :].astype(BF16)
    cps[4].wait()
    for j in range(4):
        tmpT[j] = bwo[:, j * 128:(j + 1) * 128].astype(F32)
    for d in range(DH):
        for j in range(4):
            bwop[d * H:(d + 1) * H, j * 128:(j + 1) * 128] = tmpT[j, pl.ds(d, H, stride=DH), :].astype(BF16)
    ks[:, 0:PAD, :] = jnp.zeros((4, PAD, 128), F32)
    vs[:, 0:PAD, :] = jnp.zeros((4, PAD, 128), F32)
    cps[5].wait()

    def p2(i, _):
        r = pl.multiple_of(i * BM, BM)
        xa = ax[pl.ds(r, BM), :]
        xb = xa
        gate = jax.nn.sigmoid(jnp.sum(xa.astype(F32) * gw[...].astype(F32), axis=1, keepdims=True))
        qkv = lax.dot_general(xb, wpT[...], NT, preferred_element_type=F32)
        qs[...] = qkv[:, 0:D] * (DH ** -0.5)
        for j in range(4):
            ks[j, pl.ds(r + PAD, BM), :] = qkv[:, D + j * 128:D + (j + 1) * 128]
            vs[j, pl.ds(r + PAD, BM), :] = qkv[:, 2 * D + j * 128:2 * D + (j + 1) * 128]

        def att(c, _):
            lr = pl.multiple_of(c * CH, CH)
            q = qs[pl.ds(lr, CH), :]
            base = r + lr + PAD
            pos = lax.broadcasted_iota(jnp.int32, (CH, 128), 0) + (r + lr)
            lg = []
            for w in range(W):
                k = jnp.concatenate([ks[j, pl.ds(base - 2 * w, CH), :] for j in range(4)], axis=1)
                p = q * k
                t = (p[:, 0:128] + p[:, 128:256]) + (p[:, 256:384] + p[:, 384:512])
                t = t + pltpu.roll(t, 64, 1)
                t = t + pltpu.roll(t, 32, 1)
                if w > 0:
                    t = jnp.where(pos >= 2 * w, t, -1e9)
                lg.append(t)
            m = lg[0]
            for w in range(1, W):
                m = jnp.maximum(m, lg[w])
            e = [jnp.exp(l - m) for l in lg]
            s = e[0]
            for w in range(1, W):
                s = s + e[w]
            inv = 1.0 / s
            o = None
            for w in range(W):
                v = jnp.concatenate([vs[j, pl.ds(base - 2 * w, CH), :] for j in range(4)], axis=1)
                a = e[w] * inv
                a4 = jnp.concatenate([a, a, a, a], axis=1)
                o = a4 * v if o is None else o + a4 * v
            ob[pl.ds(lr, CH), :] = o
            return 0
        lax.fori_loop(0, BM // CH, att, 0)

        q = jnp.dot(xa, awqkv[:, 0:D], preferred_element_type=F32)
        pq = _phi(q)
        pqb = pq.astype(BF16)
        den = jnp.concatenate(
            [jnp.dot(pqb[:, j * 128:(j + 1) * 128], zblk[j * 128:(j + 1) * 128, :],
                     preferred_element_type=F32) for j in range(4)], axis=1)
        oa = (pq / (den + 1e-6) * gate).astype(BF16)
        obb = (ob[...] * (1.0 - gate)).astype(BF16)
        res = jnp.dot(oa, mmat[...], preferred_element_type=F32)
        res = res + jnp.dot(obb, bwop[...], preferred_element_type=F32)
        outv[pl.ds(r, BM), :] = res.astype(outv.dtype)
        pltpu.make_async_copy(outv.at[pl.ds(r, BM), :], out_h.at[pl.ds(r, BM), :], osem.at[i]).start()
        return 0

    lax.fori_loop(0, S // BM, p2, 0)
    for i in range(S // BM):
        pltpu.make_async_copy(outv.at[pl.ds(i * BM, BM), :], out_h.at[pl.ds(i * BM, BM), :], osem.at[i]).wait()


@jax.jit
def pallas_gated_mix__linear_attn_block__sliding_local_dilated__prompt_kernel(
        A_x, A_wqkv, A_wo, B_x, B_wqkv, B_wo, gate_w):
    anyspec = pl.BlockSpec(memory_space=pl.ANY)
    V = pltpu.VMEM
    out = pl.pallas_call(
        _kernel,
        out_shape=jax.ShapeDtypeStruct((S, D), A_x.dtype),
        in_specs=[anyspec] * 7,
        out_specs=anyspec,
        scratch_shapes=[
            V((S, D), BF16), V((S, D), BF16), V((D, 3 * D), BF16), V((D, D), BF16),
            V((D, 3 * D), BF16), V((D, D), BF16), V((1, D), BF16), V((S, D), BF16),
            V((D, D), BF16), V((4, D, 128), F32), V((3 * D, D), BF16), V((D, D), BF16),
            V((D, D), F32), V((D, 128), BF16), V((D, D), BF16),
            V((BM, D), F32), V((4, S + PAD, 128), F32), V((4, S + PAD, 128), F32), V((BM, D), F32),
            pltpu.SemaphoreType.DMA((7,)), pltpu.SemaphoreType.DMA((S // BM,)),
        ],
        compiler_params=pltpu.CompilerParams(vmem_limit_bytes=100 * 1024 * 1024),
    )(A_x.reshape(S, D), A_wqkv, A_wo, B_x.reshape(S, D), B_wqkv, B_wo, gate_w.reshape(1, D))
    return out.reshape(1, S, D)
```

```python
import jax
import jax.numpy as jnp
from jax import lax
import jax.experimental.pallas as pl
import jax.experimental.pallas.tpu as pltpu

S, D, H, DH, W = 2048, 512, 32, 16, 8
BM1 = 512
BM = 256
CH = 32
PAD = 16
F32, BF16 = jnp.float32, jnp.bfloat16
NT = (((1,), (1,)), ((), ()))


def _phi(t):
    return jnp.where(t > 0, t + 1.0, jnp.exp(t)) + 1e-6


def _rcp(d):
    r = pl.reciprocal(d, approx=True)
    return r * (2.0 - d * r)


def _kernel(ax_h, awqkv_h, awo_h, bx_h, bwqkv_h, bwo_h, gw_h, out_h,
            ax, bx, awqkv, awo, bwqkv, bwo, gw, outv,
            wkT, tmpT, wpT, bwop, gacc, zblk, mmat, qs, ks, vs, zacc, pqs, gs, obs,
            sems, osem, xsem, wsem):
    cps = [
        None, None,
        pltpu.make_async_copy(awo_h, awo, sems.at[2]),
        pltpu.make_async_copy(bwqkv_h, bwqkv, sems.at[3]),
        pltpu.make_async_copy(bwo_h, bwo, sems.at[4]),
        pltpu.make_async_copy(gw_h, gw, sems.at[5]),
    ]
    xc = [pltpu.make_async_copy(ax_h.at[i * 512:(i + 1) * 512], ax.at[i * 512:(i + 1) * 512], xsem.at[i]) for i in range(4)]
    wc = [pltpu.make_async_copy(awqkv_h.at[:, t * D:(t + 1) * D], awqkv.at[:, t * D:(t + 1) * D], wsem.at[t]) for t in range(3)]
    for c in (wc[1], xc[0]):
        c.start()
    wc[1].wait()
    for c in (cps[5], wc[0], xc[1]):
        c.start()
    wkT[...] = awqkv[:, D:2 * D].astype(F32).T.astype(BF16)
    xc[0].wait()
    cps[3].start()
    NB = S // BM
    rows = lambda i: slice(i * BM, (i + 1) * BM)
    cols = lambda j: slice(j * 128, (j + 1) * 128)

    OG = {3: 0, 6: 4, 7: 7}

    def ocp(i):
        sl = slice(OG[i] * BM, (i + 1) * BM)
        return pltpu.make_async_copy(outv.at[sl, :], out_h.at[sl, :], osem.at[i])

    def jobA(i):
        if i % 2 == 0 and i > 0:
            xc[i // 2].wait()
        if i == 2:
            for c in (cps[4], xc[2], xc[3], wc[2], cps[2]):
                c.start()
        xb = ax[rows(i), :]
        pk = []
        for h in range(2):
            pk.append(_phi(lax.dot_general(wkT[h * 256:(h + 1) * 256, :], xb, NT, preferred_element_type=F32)))
            yield
        pkT = jnp.concatenate(pk, axis=0)
        g = jnp.dot(pkT.astype(BF16), xb, preferred_element_type=F32)
        zp = pkT[:, 0:128]
        for j in range(1, BM // 128):
            zp = zp + pkT[:, cols(j)]
        if i == 0:
            gacc[...] = g
            zacc[...] = zp
        else:
            gacc[...] += g
            zacc[...] += zp
        yield
        if i == 0:
            cps[5].wait()
            wc[0].wait()
        for h in range(2):
            q = jnp.dot(xb, awqkv[:, h * 256:(h + 1) * 256], preferred_element_type=F32)
            pqs[rows(i), h * 256:(h + 1) * 256] = _phi(q).astype(BF16)
            if h == 0:
                yield
        gate = jax.nn.sigmoid(jnp.sum(xb.astype(F32) * gw[...].astype(F32).reshape(1, D), axis=1, keepdims=True))
        gs[rows(i), :] = jnp.broadcast_to(gate, (BM, 128))
        yield

    def jobPerm():
        cps[3].wait()
        for t in range(3):
            wt = bwqkv[:, t * D:(t + 1) * D].astype(F32).T
            for j in range(4):
                tmpT[t, j] = wt[:, cols(j)]
            yield
            for d in range(DH):
                for j in range(4):
                    wpT[t * D + d * H:t * D + (d + 1) * H, cols(j)] = tmpT[t, j, pl.ds(d, H, stride=DH), :].astype(BF16)
                if d % 4 == 3:
                    yield
        cps[4].wait()
        for j in range(4):
            tmpT[3, j] = bwo[:, cols(j)].astype(F32)
        for d in range(DH):
            for j in range(4):
                bwop[d * H:(d + 1) * H, cols(j)] = tmpT[3, j, pl.ds(d, H, stride=DH), :].astype(BF16)
            if d % 4 == 3:
                yield
        ks[:, 0:PAD, :] = jnp.zeros((4, PAD, 128), F32)
        vs[:, 0:PAD, :] = jnp.zeros((4, PAD, 128), F32)

    def jobP(i):
        xb = ax[rows(i), :]
        for t, dst in enumerate((qs, ks, vs)):
            for h in range(2):
                y = lax.dot_general(xb, wpT[t * D + h * 256:t * D + (h + 1) * 256, :], NT, preferred_element_type=F32)
                if t == 0:
                    y = y * (DH ** -0.5 * 1.4426950408889634)
                for j in range(2):
                    dst[2 * h + j, PAD + i * BM:PAD + (i + 1) * BM, :] = y[:, cols(j)]
                yield

    def jobT(i):
        for c in range(BM // CH):
            r0 = i * BM + c * CH
            base = r0 + PAD
            q = [qs[j, base:base + CH, :] for j in range(4)]
            lg = []
            for w in range(W):
                p = [q[j] * ks[j, base - 2 * w:base - 2 * w + CH, :] for j in range(4)]
                t = (p[0] + p[1]) + (p[2] + p[3])
                t = t + pltpu.roll(t, 64, 1)
                t = t + pltpu.roll(t, 32, 1)
                if r0 < 2 * w:
                    pos = lax.broadcasted_iota(jnp.int32, (CH, 128), 0) + r0
                    t = jnp.where(pos >= 2 * w, t, -1e9)
                lg.append(t)
            m = lg[0]
            for w in range(1, W):
                m = jnp.maximum(m, lg[w])
            e = [jnp.exp2(l - m) for l in lg]
            s = e[0]
            for w in range(1, W):
                s = s + e[w]
            inv = (1.0 - gs[r0:r0 + CH, :]) * _rcp(s)
            a = [x * inv for x in e]
            yield
            for j in range(4):
                o = a[0] * vs[j, base:base + CH, :]
                for w in range(1, W):
                    o = o + a[w] * vs[j, base - 2 * w:base - 2 * w + CH, :]
                obs[r0:r0 + CH, cols(j)] = o.astype(BF16)
            yield

    def jobM():
        cps[2].wait()
        wc[2].wait()
        z = jnp.sum(zacc[...], axis=1, keepdims=True)
        ri = lax.broadcasted_iota(jnp.int32, (128, 128), 0) // DH
        ci = lax.broadcasted_iota(jnp.int32, (128, 128), 1) // DH
        bd = ri == ci
        for j in range(4):
            sl = cols(j)
            zblk[sl, :] = jnp.where(bd, z[sl, :], 0.0).astype(BF16)
            kv = jnp.dot(gacc[sl, :].astype(BF16), awqkv[:, 2 * D + j * 128:2 * D + (j + 1) * 128],
                         preferred_element_type=F32)
            kv = jnp.where(bd, kv, 0.0).astype(BF16)
            mmat[sl, :] = jnp.dot(kv, awo[sl, :], preferred_element_type=F32).astype(BF16)
            yield

    def jobO(i):
        pqb = pqs[rows(i), :]
        den = jnp.concatenate(
            [jnp.dot(pqb[:, cols(j)], zblk[cols(j), :], preferred_element_type=F32) for j in range(4)], axis=1)
        g = gs[rows(i), :]
        g4 = jnp.concatenate([g] * 4, axis=1)
        oa = (pqb.astype(F32) * (_rcp(den + 1e-6) * g4)).astype(BF16)
        yield
        for h in range(2):
            hs = slice(h * 256, (h + 1) * 256)
            res = jnp.dot(obs[rows(i), :], bwop[:, hs], preferred_element_type=F32)
            yield
            res = res + jnp.dot(oa, mmat[:, hs], preferred_element_type=F32)
            outv[rows(i), hs] = res.astype(outv.dtype)
            if h == 0:
                yield
        if i in OG:
            ocp(i).start()
        yield

    def chain(*gs_):
        for g in gs_:
            yield from g

    def par(main, side, ratio):
        acc = 0.0
        done = False
        for _ in main:
            acc += ratio
            while acc >= 1 and not done:
                acc -= 1
                try:
                    next(side)
                except StopIteration:
                    done = True
        for _ in side:
            pass

    for _ in chain(jobA(0), jobA(1)):
        pass
    par(jobPerm(), chain(jobA(2), jobA(3)), 10 / 18)
    for _ in chain(jobP(0)):
        pass
    side = {0: [jobP(1), jobA(4)], 1: [jobP(2), jobA(5)], 2: [jobP(3), jobA(6)], 3: [jobP(4), jobA(7), jobM()],
            4: [jobP(5), jobO(0), jobO(1)], 5: [jobP(6), jobO(2), jobO(3)], 6: [jobP(7), jobO(4), jobO(5)],
            7: [jobO(6)]}
    cnt = {0: 11, 1: 11, 2: 11, 3: 15, 4: 16, 5: 16, 6: 16, 7: 5}
    for i in range(NB):
        par(jobT(i), chain(*side[i]), cnt[i] / (2 * BM // CH))
    for _ in jobO(7):
        pass
    for i in OG:
        ocp(i).wait()


@jax.jit
def pallas_gated_mix__linear_attn_block__sliding_local_dilated__prompt_kernel(
        A_x, A_wqkv, A_wo, B_x, B_wqkv, B_wo, gate_w):
    anyspec = pl.BlockSpec(memory_space=pl.ANY)
    V = pltpu.VMEM
    out = pl.pallas_call(
        _kernel,
        out_shape=jax.ShapeDtypeStruct((S, D), A_x.dtype),
        in_specs=[anyspec] * 7,
        out_specs=anyspec,
        scratch_shapes=[
            V((S, D), BF16), V((S, D), BF16), V((D, 3 * D), BF16), V((D, D), BF16),
            V((D, 3 * D), BF16), V((D, D), BF16), V((D,), BF16), V((S, D), BF16),
            V((D, D), BF16), V((4, 4, D, 128), F32), V((3 * D, D), BF16), V((D, D), BF16),
            V((D, D), F32), V((D, 128), BF16), V((D, D), BF16),
            V((4, S + PAD, 128), F32), V((4, S + PAD, 128), F32), V((4, S + PAD, 128), F32),
            V((D, 128), F32), V((S, D), BF16), V((S, 128), F32), V((S, D), BF16),
            pltpu.SemaphoreType.DMA((7,)), pltpu.SemaphoreType.DMA((S // BM,)),
            pltpu.SemaphoreType.DMA((4,)), pltpu.SemaphoreType.DMA((3,)),
        ],
        compiler_params=pltpu.CompilerParams(vmem_limit_bytes=100 * 1024 * 1024, flags={"XLA_TPU_FORCE_LP_LLO_SCHEDULER": True}),
    )(A_x.reshape(S, D), A_wqkv, A_wo, B_x.reshape(S, D), B_wqkv, B_wo, gate_w)
    return out.reshape(1, S, D)
```
